```python
import os as _os
_os.environ.setdefault("JAX_PLATFORMS", "cpu")
import jax
import jax.numpy as jnp

def _softmax(x, axis=-1):
    return jax.nn.softmax(x, axis=axis)
def _gelu(x):
    return jax.nn.gelu(x, approximate=True)
def _silu(x):
    return jax.nn.silu(x)
def _sigmoid(x):
    return jax.nn.sigmoid(x)
def _layernorm(x, axis=-1, eps=1e-5):
    m = jnp.mean(x, axis=axis, keepdims=True)
    v = jnp.var(x, axis=axis, keepdims=True)
    return (x - m) / jnp.sqrt(v + eps)
def _scatter_add(tgt, idx, src, axis=0):
    return tgt.at[idx].add(src)
def _segment_sum(src, seg, n):
    return jax.ops.segment_sum(src, seg, n)
class _Rng:
    def __init__(self, key):
        self._k = key
    def _next(self):
        self._k, sub = jax.random.split(self._k)
        return sub
    def normal(self, shape):
        return jax.random.normal(self._next(), shape, dtype=jnp.bfloat16)
    def randint(self, lo, hi, shape):
        return jax.random.randint(self._next(), shape, lo, hi, dtype=jnp.int32)
    def uniform(self, shape, lo=0.0, hi=1.0):
        return jax.random.uniform(self._next(), shape, jnp.bfloat16, lo, hi)
    def permutation(self, n):
        return jax.random.permutation(self._next(), n)


kernel_name = 'standalone__linear_kernel_hedgehog__prompt'

def setup_inputs():
    _rng = _Rng(jax.random.key(int.from_bytes(__import__("os").urandom(4), "little")))
    _w = (lambda a: (lambda t: t.astype(jnp.bfloat16) if jnp.issubdtype(t.dtype, jnp.floating) else t)(jnp.asarray(a)))
    B, S, D, H = 1, 2048, 1024, 32
    Dh = D // H
    return {
        "x": _w((lambda *s: _rng.normal(s) * 0.4)(B, S, D)),
        "wqkv": _w((lambda *s: _rng.normal(s) * 0.4)(D, 3 * D)),
        "w_phi": _w((lambda *s: _rng.normal(s) * 0.4)(H, Dh, Dh) * (Dh ** -0.5)),
        "wo": _w((lambda *s: _rng.normal(s) * 0.05)(D, D)),
    }

def reference(x, wqkv, w_phi, wo):
    B, S, D = x.shape
    H = 32; Dh = D // H
    qkv = (lambda x, *d: x.transpose(*d))((x @ wqkv).reshape(B, S, 3, H, Dh), 2, 0, 3, 1, 4)
    q, k, v = qkv[0], qkv[1], qkv[2]
    pq = jnp.einsum("bhsd,hdf->bhsf", q, w_phi)
    pk = jnp.einsum("bhsd,hdf->bhsf", k, w_phi)
    phi_q = jnp.concatenate([_softmax(pq, axis=-1), _softmax(-pq, axis=-1)], axis=-1)
    phi_k = jnp.concatenate([_softmax(pk, axis=-1), _softmax(-pk, axis=-1)], axis=-1)
    kv = jnp.einsum("bhsf,bhsd->bhfd", phi_k, v)
    z  = jnp.einsum("bhsf->bhf", phi_k)
    num = jnp.einsum("bhqf,bhfd->bhqd", phi_q, kv)
    den = jnp.einsum("bhqf,bhf->bhq", phi_q, z)[..., None] + 1e-6
    o = num / den
    return (lambda x, *d: x.transpose(*d))(o, 0, 2, 1, 3).reshape(B, S, D) @ wo
```

```python
import functools, math
import jax, jax.numpy as jnp
from jax import lax
from jax.experimental import pallas as pl
from jax.experimental.pallas import tpu as pltpu

bf = jnp.bfloat16; f32 = jnp.float32; u32 = jnp.uint32
LOG2E = 1.4426950408889634
NT = (((1,), (1,)), ((), ()))
NN = (((1,), (0,)), ((), ()))

def rcp(x):
    r = pl.reciprocal(x, approx=True)
    return r * (2.0 - x * r)

def dual_softmax_T(p, nh):
    ts = p.shape[1]
    p3 = p.reshape(nh, 32, ts)
    mx = jnp.max(p3, axis=1, keepdims=True)
    mn = jnp.min(p3, axis=1, keepdims=True)
    ep = jnp.exp2(p3 - mx)
    en = jnp.exp2(mn - p3)
    rp = rcp(jnp.sum(ep, axis=1, keepdims=True))
    rn = rcp(jnp.sum(en, axis=1, keepdims=True))
    return ep * rp, en * rn

def a_combos(a11, a12, a21, a22):
    return [a11 + a22, a21 + a22, a11, a22, a11 + a12, a21 - a11, a12 - a22]
def b_combos(b11, b12, b21, b22):
    return [b11 + b22, b11, b12 - b22, b21 - b11, b22, b11 + b12, b21 + b22]
CONTRIB = {0: ((0, 1), (3, 1)), 1: ((2, 1), (3, -1)), 2: ((1, 1), (3, 1)), 3: ((0, 1), (2, 1)),
           4: ((0, -1), (1, 1)), 5: ((3, 1),), 6: ((0, 1),)}
def strassen_c(m, order, hooks):
    c = [None] * 4
    for n, i in enumerate(order):
        mi = m(i)
        for j, s in CONTRIB[i]:
            if c[j] is None: c[j] = (mi, s)
            else:
                a, sa = c[j]
                if sa > 0: c[j] = ((a + mi) if s > 0 else (a - mi), 1)
                else: c[j] = ((mi - a) if s > 0 else None, 1)
        for h in hooks.get(n + 1, ()): h()
    return [x[0] for x in c]
def pk(x): return pltpu.bitcast(x.astype(bf), u32)
def unpk(x): return pltpu.bitcast(x, bf)
def pki(a, b): return pltpu.pack_elementwise([a, b], packed_dtype=bf)
def pk_heads(x):
    n = x.shape[0] // 32; c = x.shape[1]
    x4 = x.reshape(n, 2, 16, c)
    return pki(x4[:, 0].reshape(n * 16, c), x4[:, 1].reshape(n * 16, c))
def upi(x, i): return pltpu.unpack_elementwise(x, index=i, packed_dtype=bf, unpacked_dtype=f32)
def cat1(xs): return jnp.concatenate(xs, axis=1) if len(xs) > 1 else xs[0]

def make(S=2048, D=1024, H=32, TS=512, RB=16, order=(0,6,3,4,1,2,5), oorder=(0,6,3,4,1,2,5), lead=2,
         wp=2, fp=5, olag=5, dmap=3, xpp=3, qfp=3, dbg=''):
    Dh = D // H
    NG = D // 128
    NP = NG // 2
    NTILE = S // TS
    NL = TS // 128
    HS = TS // 2; HD = D // 2; KT = HD // 128
    NSTEP = NTILE * NP
    def kernel(x_hbm, w_hbm, wphi_hbm, wo_hbm, out_hbm,
               x_v, w_v, wphi_v, wo_v, ws_v, xs_v, kvT_v, z_v, wos_v, of_v, out_v, bd_v, sems, osems):
        cps = {}
        n = [0]
        def start(key, src, dst):
            if 'nodma' in dbg:
                class _N:
                    def wait(self): pass
                cps[key] = _N(); return
            c = pltpu.make_async_copy(src, dst, sems.at[n[0]]); n[0] += 1
            c.start(); cps[key] = c
        def wchunk(key, which, p0, np_):
            start(key, w_hbm.at[:, pl.ds(which * D + p0 * 256, np_ * 256)], w_v[which].at[:, pl.ds(p0 * 256, np_ * 256)])
        start('x0', x_hbm.at[pl.ds(0, TS), :], x_v[0])
        wchunk('v0', 2, 0, 1)
        wchunk('v1', 2, 1, 1)
        start('phi', wphi_hbm, wphi_v)
        wchunk('k0', 1, 0, 1)
        wchunk('v2', 2, 2, 1)
        wchunk('k1', 1, 1, 1)
        wchunk('v3', 2, 3, 1)
        wchunk('k23', 1, 2, 2)
        for t in range(1, NTILE):
            start(('x', t), x_hbm.at[pl.ds(t * TS, TS), :], x_v[t])
        wchunk('q', 0, 0, 4)
        start('wo', wo_hbm, wo_v)
        late = []
        def wait(*keys):
            for k in keys:
                if dbg == 'all' or (isinstance(k, str) and k in dbg.split(',')): late.append(cps[k])
                else: cps[k].wait()

        rr = lax.broadcasted_iota(jnp.int32, (128, 128), 0)
        cc = lax.broadcasted_iota(jnp.int32, (128, 128), 1)
        bdmask = (rr // Dh) == (cc // Dh)
        rk = lax.broadcasted_iota(jnp.int32, (64, 128), 0)
        ck = lax.broadcasted_iota(jnp.int32, (64, 128), 1)
        kvmask = (rk // 32) == (ck // 64)
        vT = {}; kvb = {}; osd = {}
        def build_bd():
            for g in range(NG):
                xg = wphi_v[g*128:(g+1)*128, :].astype(f32).T
                bd_v[g] = pk(jnp.where(bdmask, jnp.concatenate([xg] * 4, axis=0), 0.0))

        def store_w(which, p, c, a11, a12, a21, a22):
            cs = a_combos(a11, a12, a21, a22)
            for i in range(7):
                ws_v[which][p][i, :, c*128:(c+1)*128] = pk_heads(cs[i])
        def fold(which, p):
            if 'nofold' in dbg: return
            g0, g1 = 2 * p, 2 * p + 1
            for c in range(KT):
                def f(g, r0):
                    return lax.dot_general(unpk(bd_v[g]), w_v[which][r0:r0+128, g*128:(g+1)*128], NT, preferred_element_type=f32) * LOG2E
                store_w(which, p, c, f(g0, c*128), f(g0, HD + c*128), f(g1, c*128), f(g1, HD + c*128))
        def vtrans(p):
            if 'novt' in dbg: return
            g0, g1 = 2 * p, 2 * p + 1
            for c in range(KT):
                def f(g, r0): return w_v[2][r0:r0+128, g*128:(g+1)*128].astype(f32).T
                store_w(2, p, c, f(g0, c*128), f(g0, HD + c*128), f(g1, c*128), f(g1, HD + c*128))
        def xprep(t, part=0, nparts=1):
            if 'noxp' in dbg: return
            nb = HS // RB
            for b in range(part * nb // nparts, (part + 1) * nb // nparts):
                r = b * RB
                b11 = pltpu.bitcast(x_v[t][r:r+RB, :HD], u32); b12 = pltpu.bitcast(x_v[t][HS+r:HS+r+RB, :HD], u32)
                b21 = pltpu.bitcast(x_v[t][r:r+RB, HD:], u32); b22 = pltpu.bitcast(x_v[t][HS+r:HS+r+RB, HD:], u32)
                ce = b_combos(upi(b11, 0), upi(b12, 0), upi(b21, 0), upi(b22, 0))
                co = b_combos(upi(b11, 1), upi(b12, 1), upi(b21, 1), upi(b22, 1))
                for i in range(7):
                    xs_v[t][i, r//2:(r+RB)//2, :] = b11 if i == 1 else b22 if i == 4 else pki(ce[i], co[i])
        def proj(which, t, p, hooks):
            def m(i):
                return lax.dot_general(unpk(ws_v[which][p][i]), unpk(xs_v[t][i]), NT, preferred_element_type=f32)
            c11, c12, c21, c22 = strassen_c(m, order, hooks)
            return [cat1([c11, c12]), cat1([c21, c22])]
        def phis(p):
            pos, neg = dual_softmax_T(p, 4)
            return [jnp.concatenate([pos[2*j], neg[2*j], pos[2*j+1], neg[2*j+1]], axis=0) for j in range(2)]
        def stage_v(i, hooks={}):
            t, p = divmod(i, NP)
            vs = proj(2, t, p, hooks)
            for e in range(2):
                vT[i, e] = vs[e].astype(bf)
        def stage_k(i, hooks={}):
            t, p = divmod(i, NP)
            ks = proj(1, t, p, hooks)
            out = []
            for e in range(2):
                g = 2 * p + e
                ph = []
                for j, phi in enumerate(phis(ks[e])):
                    zs = phi[:, 0:128]
                    for l in range(1, NL):
                        zs = zs + phi[:, l*128:(l+1)*128]
                    if t == 0 or 'noz' in dbg: z_v[g][j] = zs
                    else: z_v[g][j] += zs
                    ph.append(phi.astype(bf))
                out.append(ph)
            return out
        def stage_kv(i, phs):
            t, p = divmod(i, NP)
            for e in range(2):
                g = 2 * p + e
                for j in range(2):
                    kv = lax.dot_general(vT[i, e][j*64:(j+1)*64], phs[e][j], NT, preferred_element_type=f32)
                    if t == 0: kvT_v[g][j] = kv
                    elif t == NTILE - 1:
                        kvb[g, j] = jnp.where(kvmask, kvT_v[g][j] + kv, 0.0).astype(bf)
                    else: kvT_v[g][j] += kv
        def stage_q(i, hooks={}):
            t, p = divmod(i, NP)
            qs = proj(0, t, p, hooks)
            out = []
            for e in range(2):
                g = 2 * p + e
                ph, rd = [], []
                for j, phi in enumerate(phis(qs[e])):
                    zb = cat1([z_v[g][j]] * NL)
                    den = jnp.sum((phi * zb).reshape(2, 64, TS), axis=1, keepdims=True) + 1e-6
                    ph.append(phi.astype(bf)); rd.append(rcp(den))
                out.append((ph, rd))
            return out
        def stage_num(i, fq):
            t, p = divmod(i, NP)
            for e in range(2):
                g = 2 * p + e
                ph, rd = fq[e]
                os_ = []
                for j in range(2):
                    nm = lax.dot_general(kvb[g, j], ph[j], NN, preferred_element_type=f32)
                    os_.append((nm.reshape(2, 32, TS) * rd[j]).reshape(64, TS))
                oT = jnp.concatenate(os_, axis=0)
                o = [oT[:, l*128:(l+1)*128].T for l in range(NL)]
                if g < KT:
                    for l in range(NL): of_v[g][l*128:(l+1)*128, :] = o[l]
                else:
                    j = g - KT
                    for l in range(NL // 2):
                        a11 = of_v[j][l*128:(l+1)*128, :]; a21 = of_v[j][HS+l*128:HS+(l+1)*128, :]
                        a12 = o[l]; a22 = o[NL // 2 + l]
                        cs = a_combos(a11, a12, a21, a22)
                        for c in range(7): osd[t, c, l, j] = cs[c].astype(bf)
        def wo_prep(part=0, nparts=1):
            nb = HD // 32
            for b in range(part * nb // nparts, (part + 1) * nb // nparts):
                r = b * 32
                b11 = wo_v[r:r+32, :HD]; b12 = wo_v[r:r+32, HD:]
                b21 = wo_v[HD+r:HD+r+32, :HD]; b22 = wo_v[HD+r:HD+r+32, HD:]
                cs = b_combos(b11.astype(f32), b12.astype(f32), b21.astype(f32), b22.astype(f32))
                for c in range(7):
                    wos_v[c, r//2:(r+32)//2, :] = pk_heads(cs[c])
        ocps = []
        def outp(ci, hooks={}):
            t, m = divmod(ci, 4)
            ms, ns = divmod(m, 2)
            def mm(i):
                a = cat1([osd[t, i, ms, j] for j in range(KT)]); b = unpk(wos_v[i, :, ns*256:(ns+1)*256])
                return lax.dot_general(a, b, NN, preferred_element_type=f32)
            c11, c12, c21, c22 = strassen_c(mm, oorder, hooks)
            out_v[t][ms*128:(ms+1)*128, ns*256:(ns+1)*256] = c11.astype(bf)
            out_v[t][ms*128:(ms+1)*128, HD+ns*256:HD+(ns+1)*256] = c12.astype(bf)
            out_v[t][HS+ms*128:HS+(ms+1)*128, ns*256:(ns+1)*256] = c21.astype(bf)
            out_v[t][HS+ms*128:HS+(ms+1)*128, HD+ns*256:HD+(ns+1)*256] = c22.astype(bf)
        def outdma(t, r0, nr):
            if 'noout' in dbg: return
            cp = pltpu.make_async_copy(out_v[t].at[pl.ds(r0, nr), :], out_hbm.at[pl.ds(t * TS + r0, nr), :], osems.at[len(ocps)])
            cp.start(); ocps.append(cp)
        P = functools.partial

        if 'p2only' not in dbg:
            wait('x0')
            xprep(0)
            wait('v0')
            vtrans(0)
            stage_v(0, {wp + 2: [P(wait, 'v1'), P(vtrans, 1)]})
        if 'p2only' in dbg: pass
        elif lead == 2:
            stage_v(1, {wp: [P(wait, 'phi', 'k0'), build_bd], fp: [P(fold, 1, 0)]})
        else:
            wait('phi', 'k0'); build_bd(); fold(1, 0)
        for i in range(NSTEP if 'p2only' not in dbg else 0):
            t, p = divmod(i, NP)
            hk = {}; hv = {}
            def add(h, pos, f): h.setdefault(pos, []).append(f)
            if i == 0:
                add(hk, wp, P(wait, 'v2', 'k1')); add(hk, wp, P(vtrans, 2)); add(hk, fp, P(fold, 1, 1))
            if i == 1:
                add(hk, wp, P(wait, 'v3', 'k23')); add(hk, wp, P(vtrans, 3)); add(hk, fp, P(fold, 1, 2)); add(hv, fp, P(fold, 1, 3))
                add(hv, wp, P(wait, *[('x', tt) for tt in range(1, NTILE)]))
                add(hv, 6, P(xprep, 1, 0, 2))
            if i == 2: add(hk, xpp, P(xprep, 1, 1, 2))
            if i == 5: add(hk, wp, P(wait, 'q', 'wo'))
            for tt in range(2, NTILE):
                j = i - (NP * tt - lead - 3)
                if 0 <= j < 4: add(hk, xpp, P(xprep, tt, j, 4))
            if 8 <= i < 12: add(hv, xpp, P(wo_prep, i - 8, 4))
            if t == NTILE - 1: add(hk, qfp, P(fold, 0, p))
            phs = stage_k(i, hk)
            if i + lead < NSTEP: stage_v(i + lead, hv)
            else:
                for fs in hv.values():
                    for f in fs: f()
            stage_kv(i, phs)
        for g in range(NG):
            for j in range(2):
                zt = jnp.sum(z_v[g][j], axis=1, keepdims=True)
                z_v[g][j] = jnp.broadcast_to(zt, (128, 128))

        if 'p1only' in dbg:
            out_v[1][0:16, :] = out_v[0][0:16, :]
            outdma(1, 0, 16)
            for cp in ocps + late: cp.wait()
            return
        pend = None
        NCH = 4 * NTILE
        def dmas_after(ci):
            t, m = divmod(ci, 4)
            if t < NTILE - 1: return [P(outdma, t, 0, TS)] if m == 3 else []
            if m % 2 == 1:
                ms = m // 2
                return [P(outdma, t, ms * 128, 128), P(outdma, t, HS + ms * 128, 128)]
            return []
        todo = []
        for i in range(NSTEP):
            fq = stage_q(i, {dmap: todo}); todo = []
            if pend is not None: stage_num(*pend)
            pend = (i, fq)
            ci = i - olag
            if ci >= 0:
                outp(ci); todo = dmas_after(ci)
        stage_num(*pend)
        for ci in range(NSTEP - olag, NCH):
            outp(ci, {dmap: todo}); todo = dmas_after(ci)
        for f in todo: f()
        for cp in ocps + late:
            cp.wait()

    def fn(x, wqkv, w_phi, wo):
        B = x.shape[0]
        x2 = x.reshape(S, D)
        wphi2 = w_phi.reshape(H * Dh, Dh)
        VM = pltpu.VMEM
        out = pl.pallas_call(
            kernel,
            out_shape=jax.ShapeDtypeStruct((S, D), bf),
            in_specs=[pl.BlockSpec(memory_space=pl.ANY)] * 4,
            out_specs=pl.BlockSpec(memory_space=pl.ANY),
            scratch_shapes=[
                [VM((TS, D), bf) for _ in range(NTILE)], [VM((D, D), bf) for _ in range(3)], VM((H*Dh, Dh), bf),
                VM((D, D), bf), [[VM((7, 64, HD), u32) for _ in range(NP)] for _ in range(3)],
                [VM((7, HS//2, HD), u32) for _ in range(NTILE)],
                [VM((2, 64, 128), f32) for _ in range(NG)],
                [VM((2, 128, 128), f32) for _ in range(NG)],
                VM((7, HD//2, HD), u32), [VM((TS, 128), f32) for _ in range(KT)],
                [VM((TS, D), bf) for _ in range(NTILE)],
                VM((NG, 64, 128), u32),
                pltpu.SemaphoreType.DMA((14,)), pltpu.SemaphoreType.DMA((NTILE + 4,)),
            ],
            compiler_params=pltpu.CompilerParams(vmem_limit_bytes=100 << 20),
        )(x2, wqkv, wphi2, wo)
        return out.reshape(B, S, D)
    return fn


@jax.jit
def pallas_standalone__linear_kernel_hedgehog__prompt_kernel(x, wqkv, w_phi, wo):
    B, S, D = x.shape
    return make(S=S, D=D, H=w_phi.shape[0], wp=3)(x, wqkv, w_phi, wo)
```

```python
import functools

import jax
import jax.numpy as jnp
from jax import lax
import jax.experimental.pallas as pl
import jax.experimental.pallas.tpu as pltpu

bf16 = jnp.bfloat16
f32 = jnp.float32
LOG2E = 1.4426950408889634
EPS = 1e-6
NT = (((1,), (1,)), ((), ()))
NN = (((1,), (0,)), ((), ()))
DH = 32
TS = 512
LANE = 128
P = functools.partial


def _dot(a, b, dims):
    return lax.dot_general(a, b, dims, preferred_element_type=f32)


def _cat(xs, axis):
    return jnp.concatenate(xs, axis=axis)


def _rcp(x):
    r = pl.reciprocal(x, approx=True)
    return r * (2.0 - x * r)


def _features(p):
    p3 = p.reshape(4, DH, TS)
    mx = jnp.max(p3, axis=1, keepdims=True)
    mn = jnp.min(p3, axis=1, keepdims=True)
    ep = jnp.exp2(p3 - mx)
    en = jnp.exp2(mn - p3)
    pos = ep * _rcp(jnp.sum(ep, axis=1, keepdims=True))
    neg = en * _rcp(jnp.sum(en, axis=1, keepdims=True))
    return [_cat([pos[2 * j], neg[2 * j], pos[2 * j + 1], neg[2 * j + 1]], 0) for j in range(2)]


def _lhs_ops(a11, a12, a21, a22):
    return [a11 + a22, a21 + a22, a11, a22, a11 + a12, a21 - a11, a12 - a22]


def _rhs_ops(b11, b12, b21, b22):
    return [b11 + b22, b11, b12 - b22, b21 - b11, b22, b11 + b12, b21 + b22]


_ORDER = (0, 6, 3, 4, 1, 2, 5)
_CONTRIB = {0: ((0, 1), (3, 1)), 1: ((2, 1), (3, -1)), 2: ((1, 1), (3, 1)), 3: ((0, 1), (2, 1)),
            4: ((0, -1), (1, 1)), 5: ((3, 1),), 6: ((0, 1),)}


def _strassen(product, hooks):
    c = [None] * 4
    for n, i in enumerate(_ORDER):
        m = product(i)
        for j, sign in _CONTRIB[i]:
            if c[j] is None:
                assert sign > 0
                c[j] = m
            else:
                c[j] = c[j] + m if sign > 0 else c[j] - m
        for h in hooks.get(n + 1, ()):
            h()
    return c


def _kernel(x_hbm, w_hbm, wphi_hbm, wo_hbm, out_hbm,
            x_v, w_v, wphi_v, wo_v, out_v, in_sems, out_sems, *, S, D):
    NG = D // LANE
    NP = NG // 2
    NT_ = S // TS
    NL = TS // LANE
    HS, HD = TS // 2, D // 2
    KT = HD // LANE
    NSTEP = NT_ * NP
    Q, K, V = 0, 1, 2

    cps = {}

    def start(key, src, dst):
        cps[key] = pltpu.make_async_copy(src, dst, in_sems.at[len(cps)])
        cps[key].start()

    def w_chunk(key, which, p0, n):
        start(key, w_hbm.at[:, pl.ds(which * D + p0 * 256, n * 256)],
              w_v[which].at[:, pl.ds(p0 * 256, n * 256)])

    def x_chunk(t):
        start(('x', t), x_hbm.at[pl.ds(t * TS, TS), :], x_v[t])

    def wait(*keys):
        for k in keys:
            cps[k].wait()

    x_chunk(0)
    w_chunk('v0', V, 0, 1)
    w_chunk('v1', V, 1, 1)
    start('phi', wphi_hbm, wphi_v)
    w_chunk('k0', K, 0, 1)
    w_chunk('v2', V, 2, 1)
    w_chunk('k1', K, 1, 1)
    w_chunk('v3', V, 3, 1)
    w_chunk('k23', K, 2, 2)
    for t in range(1, NT_):
        x_chunk(t)
    w_chunk('q', Q, 0, NP)
    start('wo', wo_hbm, wo_v)

    rows = lax.broadcasted_iota(jnp.int32, (LANE, LANE), 0)
    cols = lax.broadcasted_iota(jnp.int32, (LANE, LANE), 1)
    bd_mask = (rows // DH) == (cols // DH)
    kv_mask = (rows[:64] // DH) == (cols[:64] // (2 * DH))

    bd, w_part, w_op, x_part, x_op, wo_part, wo_op = {}, {}, {}, {}, {}, {}, {}
    vT, z, kvT, kv_bd, o_lo, o_part, o_op = {}, {}, {}, {}, {}, {}, {}

    def build_bd():
        for g in range(NG):
            xg = wphi_v[g * LANE:(g + 1) * LANE, :].astype(f32).T
            bd[g] = jnp.where(bd_mask, _cat([xg] * 4, 0), 0.0).astype(bf16)

    def emit_w(which, p, c, blocks):
        for i, op in enumerate(_lhs_ops(*blocks)):
            w_part[which, p, i, c] = op
            if c == KT - 1:
                w_op[which, p, i] = _cat([w_part[which, p, i, cc] for cc in range(KT)], 1).astype(bf16)

    def w_tile(which, g, r0):
        return w_v[which][r0:r0 + LANE, g * LANE:(g + 1) * LANE]

    def fold(which, p):
        for c in range(KT):
            emit_w(which, p, c, [_dot(bd[g], w_tile(which, g, r0 + c * LANE), NT) * LOG2E
                                  for g in (2 * p, 2 * p + 1) for r0 in (0, HD)])

    def v_trans(p):
        for c in range(KT):
            emit_w(V, p, c, [w_tile(V, g, r0 + c * LANE).astype(f32).T
                             for g in (2 * p, 2 * p + 1) for r0 in (0, HD)])

    def x_prep(t, part=0, nparts=1):
        nb = HS // 16
        for b in range(part * nb // nparts, (part + 1) * nb // nparts):
            r = b * 16
            ops = _rhs_ops(x_v[t][r:r + 16, :HD].astype(f32), x_v[t][HS + r:HS + r + 16, :HD].astype(f32),
                           x_v[t][r:r + 16, HD:].astype(f32), x_v[t][HS + r:HS + r + 16, HD:].astype(f32))
            for i in (0, 2, 3, 5, 6):
                x_part[t, i, b] = ops[i]
                if b == nb - 1:
                    x_op[t, i] = _cat([x_part[t, i, bb] for bb in range(nb)], 0).astype(bf16)

    def wo_prep(part, nparts):
        nb = HD // 32
        for b in range(part * nb // nparts, (part + 1) * nb // nparts):
            r = b * 32
            ops = _rhs_ops(wo_v[r:r + 32, :HD].astype(f32), wo_v[r:r + 32, HD:].astype(f32),
                           wo_v[HD + r:HD + r + 32, :HD].astype(f32), wo_v[HD + r:HD + r + 32, HD:].astype(f32))
            for i in range(7):
                wo_part[i, b] = ops[i]
                if b == nb - 1:
                    for ns in range(2):
                        wo_op[i, ns] = _cat([wo_part[i, bb][:, ns * 256:(ns + 1) * 256]
                                             for bb in range(nb)], 0).astype(bf16)

    def proj(which, step, hooks):
        t, p = divmod(step, NP)

        def product(i):
            if i == 1:
                b = x_v[t][:HS, :HD]
            elif i == 4:
                b = x_v[t][HS:, HD:]
            else:
                b = x_op[t, i]
            return _dot(w_op[which, p, i], b, NT)

        c11, c12, c21, c22 = _strassen(product, hooks)
        return [_cat([c11, c12], 1), _cat([c21, c22], 1)]

    def stage_v(step, hooks):
        for e, v in enumerate(proj(V, step, hooks)):
            vT[step, e] = v.astype(bf16)

    def stage_k(step, hooks):
        t, p = divmod(step, NP)
        out = {}
        for e, pk in enumerate(proj(K, step, hooks)):
            for j, phi in enumerate(_features(pk)):
                key = (2 * p + e, j)
                zs = phi[:, :LANE]
                for l in range(1, NL):
                    zs = zs + phi[:, l * LANE:(l + 1) * LANE]
                z[key] = zs if t == 0 else z[key] + zs
                if t == NT_ - 1:
                    z[key] = jnp.broadcast_to(jnp.sum(z[key], axis=1, keepdims=True), (LANE, LANE))
                out[e, j] = phi.astype(bf16)
        return out

    def stage_kv(step, phi):
        t, p = divmod(step, NP)
        for e in range(2):
            for j in range(2):
                key = (2 * p + e, j)
                kv = _dot(vT[step, e][j * 64:(j + 1) * 64], phi[e, j], NT)
                kvT[key] = kv if t == 0 else kvT[key] + kv
                if t == NT_ - 1:
                    kv_bd[key] = jnp.where(kv_mask, kvT[key], 0.0).astype(bf16)

    def stage_q(step, hooks):
        p = step % NP
        out = {}
        for e, pq in enumerate(proj(Q, step, hooks)):
            for j, phi in enumerate(_features(pq)):
                zb = _cat([z[2 * p + e, j]] * NL, 1)
                den = jnp.sum((phi * zb).reshape(2, 2 * DH, TS), axis=1, keepdims=True) + EPS
                out[e, j] = (phi.astype(bf16), _rcp(den))
        return out

    def stage_num(step, feats):
        t, p = divmod(step, NP)
        for e in range(2):
            g = 2 * p + e
            oT = _cat([(_dot(kv_bd[g, j], feats[e, j][0], NN).reshape(2, DH, TS) * feats[e, j][1]).reshape(64, TS)
                       for j in range(2)], 0)
            o = [oT[:, l * LANE:(l + 1) * LANE].T for l in range(NL)]
            if g < KT:
                o_lo[g] = o
                continue
            c = g - KT
            for ms in range(NL // 2):
                ops = _lhs_ops(o_lo[c][ms], o[ms], o_lo[c][NL // 2 + ms], o[NL // 2 + ms])
                for i in range(7):
                    o_part[t, i, ms, c] = ops[i]
                    if c == KT - 1:
                        o_op[t, i, ms] = _cat([o_part[t, i, ms, cc] for cc in range(KT)], 1).astype(bf16)

    ocps = []

    def out_dma(t, r0, nr, c0, nc):
        cp = pltpu.make_async_copy(out_v[t].at[pl.ds(r0, nr), pl.ds(c0, nc)],
                                   out_hbm.at[pl.ds(t * TS + r0, nr), pl.ds(c0, nc)], out_sems.at[len(ocps)])
        cp.start()
        ocps.append(cp)

    todo = []

    def stage_out(chunk, hooks):
        t, m = divmod(chunk, 4)
        ms, ns = divmod(m, 2)
        blocks = _strassen(lambda i: _dot(o_op[t, i, ms], wo_op[i, ns], NN), hooks)
        corners = [(r, c) for r in (ms * LANE, HS + ms * LANE) for c in (ns * 256, HD + ns * 256)]
        for blk, (r0, c0) in zip(blocks, corners):
            out_v[t][r0:r0 + LANE, c0:c0 + 256] = blk.astype(bf16)
            if t == NT_ - 1:
                out_dma(t, r0, LANE, c0, 256)
        if m == 3 and t < NT_ - 1:
            todo.append(P(out_dma, t, 0, TS, 0, D))

    def take_todo():
        h = {3: list(todo)}
        todo.clear()
        return h

    hooks = {}

    def put(stage, step, pos, *fs):
        hooks.setdefault((stage, step), {}).setdefault(pos, []).extend(fs)

    put(V, 0, 4, P(wait, 'v1'), P(v_trans, 1))
    put(V, 1, 3, P(wait, 'phi', 'k0'), build_bd)
    put(V, 1, 5, P(fold, K, 0))
    put(K, 0, 3, P(wait, 'v2', 'k1'), P(v_trans, 2))
    put(K, 0, 5, P(fold, K, 1))
    put(K, 1, 3, P(wait, 'v3', 'k23'), P(v_trans, 3))
    put(K, 1, 5, P(fold, K, 2))
    put(V, 3, 5, P(fold, K, 3))
    put(K, 2, 1, P(wait, *[('x', t) for t in range(1, NT_)]))
    for j in range(3):
        put(K, 2, 1 + j, P(x_prep, 1, j, 3))
    put(K, 6, 3, P(wait, 'q', 'wo'))
    for j in range(4):
        put(K, 3 + j, 3, P(x_prep, 2, j, 4))
        put(K, 7 + j, 3, P(x_prep, 3, j, 4))
        put(V, 8 + j, 4, P(wo_prep, j, 4))
        put(V, 12 + j, 4, P(fold, Q, j))

    LEAD = 2
    wait(('x', 0))
    x_prep(0)
    wait('v0')
    v_trans(0)
    for i in range(LEAD):
        stage_v(i, hooks.get((V, i), {}))
    feats = {}
    for i in range(NSTEP):
        phi = stage_k(i, hooks.get((K, i), {}))
        if i + LEAD < NSTEP:
            stage_v(i + LEAD, hooks.get((V, i + LEAD), {}))
        else:
            feats[i + LEAD - NSTEP] = stage_q(i + LEAD - NSTEP, {})
        stage_kv(i, phi)

    OLAG = 6
    for i in range(LEAD, NSTEP):
        feats[i] = stage_q(i, take_todo())
        stage_num(i - LEAD, feats[i - LEAD])
        if i >= OLAG:
            stage_out(i - OLAG, {})
    chunk = NSTEP - OLAG
    for i in range(NSTEP - LEAD, NSTEP):
        stage_num(i, feats[i])
        if i < NSTEP - 1:
            stage_out(chunk, take_todo())
            chunk += 1
    for chunk in range(chunk, 4 * NT_):
        stage_out(chunk, take_todo())
    for cp in ocps:
        cp.wait()


@jax.jit
def pallas_standalone__linear_kernel_hedgehog__prompt_kernel(
    x: jax.Array,
    wqkv: jax.Array,
    w_phi: jax.Array,
    wo: jax.Array,
):
    B, S, D = x.shape
    H = w_phi.shape[0]
    assert B == 1 and S == 4 * TS and D == 1024 and H * DH == D and w_phi.shape[1:] == (DH, DH)
    n_tiles = S // TS
    vmem = pltpu.VMEM
    out = pl.pallas_call(
        P(_kernel, S=S, D=D),
        out_shape=jax.ShapeDtypeStruct((S, D), bf16),
        in_specs=[pl.BlockSpec(memory_space=pl.ANY)] * 4,
        out_specs=pl.BlockSpec(memory_space=pl.ANY),
        scratch_shapes=[
            [vmem((TS, D), bf16) for _ in range(n_tiles)],
            [vmem((D, D), bf16) for _ in range(3)],
            vmem((H * DH, DH), bf16),
            vmem((D, D), bf16),
            [vmem((TS, D), bf16) for _ in range(n_tiles)],
            pltpu.SemaphoreType.DMA((10 + n_tiles,)),
            pltpu.SemaphoreType.DMA((n_tiles - 1 + 16,)),
        ],
        compiler_params=pltpu.CompilerParams(vmem_limit_bytes=100 << 20),
    )(x.reshape(S, D), wqkv, w_phi.reshape(H * DH, DH), wo)
    return out.reshape(B, S, D)
```
